```python
import jax
import jax.numpy as jnp

def _softmax(x, axis=-1):
    return jax.nn.softmax(x, axis=axis)
def _gelu(x):
    return jax.nn.gelu(x, approximate=True)
def _silu(x):
    return jax.nn.silu(x)
def _sigmoid(x):
    return jax.nn.sigmoid(x)
def _layernorm(x, axis=-1, eps=1e-5):
    m = jnp.mean(x, axis=axis, keepdims=True)
    v = jnp.var(x, axis=axis, keepdims=True)
    return (x - m) / jnp.sqrt(v + eps)
def _scatter_add(tgt, idx, src, axis=0):
    return tgt.at[idx].add(src)
def _segment_sum(src, seg, n):
    return jax.ops.segment_sum(src, seg, n)
class _Rng:
    def __init__(self, key):
        self._k = key
    def _next(self):
        self._k, sub = jax.random.split(self._k)
        return sub
    def normal(self, shape):
        return jax.random.normal(self._next(), shape, dtype=jnp.bfloat16)
    def randint(self, lo, hi, shape):
        return jax.random.randint(self._next(), shape, lo, hi, dtype=jnp.int32)
    def uniform(self, shape, lo=0.0, hi=1.0):
        return jax.random.uniform(self._next(), shape, jnp.bfloat16, lo, hi)
    def permutation(self, n):
        return jax.random.permutation(self._next(), n)


kernel_name = 'sequential_preLN__linear_attn_block__moe_arch_mod__prompt'

def setup_inputs():
    _rng = _Rng(jax.random.key(int.from_bytes(__import__("os").urandom(4), "little")))
    _w = (lambda a: (lambda t: t.astype(jnp.bfloat16) if jnp.issubdtype(t.dtype, jnp.floating) else t)(jnp.asarray(a)))
    def _A_setup():
        B, S, D = 1, 2048, 1024
        return {
            "x": _w((lambda *s: _rng.normal(s) * 0.05)(B, S, D)),
            "wqkv": _w((lambda *s: _rng.normal(s) * 0.05)(D, 3 * D)),
            "wo": _w((lambda *s: _rng.normal(s) * 0.05)(D, D)),
        }
    _A_in = _A_setup()

    def _B_setup():
        B, S, D, F, C = 1, 2048, 1024, 3584, 2
        return {
            "x": _w((lambda *s: _rng.normal(s) * 0.05)(B, S, D)),
            "w_r": _w((lambda *s: _rng.normal(s) * 0.05)(D)),
            "w_gate": _w((lambda *s: _rng.normal(s) * 0.05)(D, F)),
            "w_up": _w((lambda *s: _rng.normal(s) * 0.05)(D, F)),
            "w_down": _w((lambda *s: _rng.normal(s) * 0.05)(F, D)),
        }
    _B_in = _B_setup()

    return {
        "A_x": _A_in["x"],
        "A_wqkv": _A_in["wqkv"],
        "A_wo": _A_in["wo"],
        "B_x": _B_in["x"],
        "B_w_r": _B_in["w_r"],
        "B_w_gate": _B_in["w_gate"],
        "B_w_up": _B_in["w_up"],
        "B_w_down": _B_in["w_down"],
    }

def reference(A_x, A_wqkv, A_wo, B_x, B_w_r, B_w_gate, B_w_up, B_w_down):
    def _A_ref(x, wqkv, wo):
        B, S, D = x.shape
        H = 32; Dh = D // H
        qkv = (lambda x, *d: x.transpose(*d))((x @ wqkv).reshape(B, S, 3, H, Dh), 2, 0, 3, 1, 4)
        q, k, v = qkv[0], qkv[1], qkv[2]
        phi = lambda t: jnp.where(t > 0, t + 1, jnp.exp(t)) + 1e-6
        pq, pk = phi(q), phi(k)
        kv = jnp.einsum("bhsd,bhse->bhde", pk, v)
        z = jnp.einsum("bhsd->bhd", pk)
        num = jnp.einsum("bhqd,bhde->bhqe", pq, kv)
        den = jnp.einsum("bhqd,bhd->bhq", pq, z)[..., None] + 1e-6
        o = num / den
        return (lambda x, *d: x.transpose(*d))(o, 0, 2, 1, 3).reshape(B, S, D) @ wo

    def _B_ref(x, w_r, w_gate, w_up, w_down):
        B, S, D = x.shape
        C = 2
        r = x @ w_r
        idx = jnp.argsort(-r, axis=-1)[:, :C]
        idx_e = jnp.repeat(idx.reshape(B, C, 1), D, axis=2)
        x_sel = jnp.take_along_axis(x, idx_e, axis=1)
        g = _silu(x_sel @ w_gate)
        u = x_sel @ w_up
        y = (g * u) @ w_down
        r_sel = _sigmoid(jnp.take_along_axis(r, idx, axis=1))
        y = y * r_sel.reshape(B, C, 1)
        b_off = (jnp.arange(B) * S).reshape(B, 1)
        flat_idx = (idx + b_off).reshape(B * C)
        zero = (x * 0.0).reshape(B * S, D)
        upd = _scatter_add(zero, flat_idx, y.reshape(B * C, D), axis=0)
        return x + upd.reshape(B, S, D)

    x = A_x
    h = x + _A_ref(_layernorm(x, axis=-1), A_wqkv, A_wo)
    h2 = h + _B_ref(_layernorm(h, axis=-1), B_w_r, B_w_gate, B_w_up, B_w_down)
    return h2
```

```python
import jax
import jax.numpy as jnp
from jax import lax
import jax.experimental.pallas as pl
import jax.experimental.pallas.tpu as pltpu

S, D, F, H = 2048, 1024, 3584, 32
TM = 512
NT = S // TM
NB = D // 128
f32 = jnp.float32
bf16 = jnp.bfloat16


def _ln(x):
    m = jnp.mean(x, axis=-1, keepdims=True)
    xc = x - m
    v = jnp.mean(xc * xc, axis=-1, keepdims=True)
    return xc * lax.rsqrt(v + 1e-5)


def _phi(t):
    return jnp.where(t > 0, t + 1.0, jnp.exp(t)) + 1e-6


def _top2(r, iota, big):
    m1 = jnp.max(r, axis=0, keepdims=True)
    i1 = jnp.min(jnp.where(r == m1, iota, big), axis=0, keepdims=True)
    r2 = jnp.where(iota == i1, -jnp.inf, r)
    m2 = jnp.max(r2, axis=0, keepdims=True)
    i2 = jnp.min(jnp.where(r2 == m2, iota, big), axis=0, keepdims=True)
    return m1, i1, m2, i2


def _kernel(x_hbm, wqkv_hbm, wo_hbm, wr_ref, wg_hbm, wu_hbm, wd_hbm, out_hbm,
            x_v, wqkv_v, wo_v, wg_v, wu_v, wd_v, ln1_v, wp_v, zbd_v, kv_v, z_v,
            h_v, out_v, cv_v, ci_v, sem_x, sem_w, sem_o, sem_f):
    def x_copy(i):
        return pltpu.make_async_copy(x_hbm.at[pl.ds(i * TM, TM)], x_v.at[pl.ds(i * TM, TM)], sem_x.at[i])

    def w_copy(j):
        c = (1, 2, 0)[j]
        return pltpu.make_async_copy(wqkv_hbm.at[:, pl.ds(c * D, D)], wqkv_v.at[:, pl.ds(c * D, D)], sem_w.at[j])

    wo_copy = pltpu.make_async_copy(wo_hbm, wo_v, sem_w.at[3])
    wg_copy = pltpu.make_async_copy(wg_hbm, wg_v, sem_w.at[4])
    wu_copy = pltpu.make_async_copy(wu_hbm, wu_v, sem_w.at[5])
    wd_copy = pltpu.make_async_copy(wd_hbm, wd_v, sem_w.at[6])

    def o_copy(i):
        rows = pl.ds(pl.multiple_of(i * TM, TM), TM)
        return pltpu.make_async_copy(out_v.at[rows], out_hbm.at[rows], sem_o.at[i])

    x_copy(0).start()
    w_copy(0).start()
    w_copy(1).start()
    for i in range(1, NT):
        x_copy(i).start()
    w_copy(2).start()
    wo_copy.start()
    wg_copy.start()
    wu_copy.start()
    wd_copy.start()

    kv_v[...] = jnp.zeros(kv_v.shape, f32)
    z_v[...] = jnp.zeros(z_v.shape, f32)

    x_copy(0).wait()
    w_copy(0).wait()
    w_copy(1).wait()

    def p1(i, carry):
        rows = pl.ds(pl.multiple_of(i * TM, TM), TM)

        @pl.when(i > 0)
        def _():
            x_copy(i).wait()

        ln1 = _ln(x_v[rows, :].astype(f32)).astype(bf16)
        ln1_v[rows, :] = ln1
        k = jnp.dot(ln1, wqkv_v[:, D:2 * D], preferred_element_type=f32)
        pkf = _phi(k)
        pk = pkf.astype(bf16)
        z_v[...] += jnp.sum(pk.astype(f32).reshape(TM // 8, 8, D), axis=0)
        v = jnp.dot(ln1, wqkv_v[:, 2 * D:3 * D], preferred_element_type=f32).astype(bf16)
        for j in range(NB):
            cs = slice(j * 128, (j + 1) * 128)
            kv_v[j] += lax.dot_general(pk[:, cs], v[:, cs], (((0,), (0,)), ((), ())),
                                       preferred_element_type=f32)
        return carry

    lax.fori_loop(0, NT, p1, 0)

    wo_copy.wait()
    w_copy(2).wait()
    ri = lax.broadcasted_iota(jnp.int32, (128, 128), 0) // 32
    ci = lax.broadcasted_iota(jnp.int32, (128, 128), 1) // 32
    mask = ri == ci
    zrow = jnp.sum(z_v[...], axis=0, keepdims=True)
    for j in range(NB):
        cs = slice(j * 128, (j + 1) * 128)
        kvb = jnp.where(mask, kv_v[j], 0.0).astype(bf16)
        wp_v[cs, :] = jnp.dot(kvb, wo_v[cs, :], preferred_element_type=f32).astype(bf16)
        zcol = jnp.transpose(jnp.broadcast_to(zrow[:, cs], (128, 128)))
        zbd_v[j] = jnp.where(mask, zcol, 0.0).astype(bf16)

    wr = wr_ref[...].astype(f32).reshape(1, D)

    def p2(i, carry):
        rows = pl.ds(pl.multiple_of(i * TM, TM), TM)
        q = jnp.dot(ln1_v[rows, :], wqkv_v[:, 0:D], preferred_element_type=f32)
        pq = _phi(q).astype(bf16)
        parts = []
        for j in range(NB):
            cs = slice(j * 128, (j + 1) * 128)
            den = jnp.dot(pq[:, cs], zbd_v[j], preferred_element_type=f32) + 1e-6
            parts.append((pq[:, cs].astype(f32) / den).astype(bf16))
        pqn = jnp.concatenate(parts, axis=1)
        attn = jnp.dot(pqn, wp_v[...], preferred_element_type=f32)
        h = (x_v[rows, :].astype(f32) + attn.astype(bf16).astype(f32)).astype(bf16).astype(f32)
        h_v[rows, :] = h
        ln2 = _ln(h).astype(bf16).astype(f32)
        out_v[rows, :] = (h + ln2).astype(bf16)
        o_copy(i).start()
        r = jnp.sum(ln2 * wr, axis=-1, keepdims=True).astype(bf16).astype(f32)
        iota = lax.broadcasted_iota(jnp.int32, (TM, 1), 0) + i * TM
        m1, i1, m2, i2 = _top2(r, iota, 1 << 30)
        cv_v[pl.ds(2 * i, 1), :] = jnp.broadcast_to(m1, (1, 128))
        cv_v[pl.ds(2 * i + 1, 1), :] = jnp.broadcast_to(m2, (1, 128))
        ci_v[pl.ds(2 * i, 1), :] = jnp.broadcast_to(i1, (1, 128))
        ci_v[pl.ds(2 * i + 1, 1), :] = jnp.broadcast_to(i2, (1, 128))
        return carry

    lax.fori_loop(0, NT, p2, 0)

    cvals = cv_v[...]
    cidx = ci_v[...]
    m1, i1, m2, i2 = _top2(cvals, cidx, 1 << 30)
    idx = [jnp.clip(i1[0, 0], 0, S - 1), jnp.clip(i2[0, 0], 0, S - 1)]
    rsel = [m1, m2]

    hh = [h_v[pl.ds(idx[c], 1), :] for c in range(2)]
    row16 = lax.broadcasted_iota(jnp.int32, (16, D), 0)
    h16 = jnp.where(row16 == 0, hh[0], jnp.where(row16 == 1, hh[1], 0.0))
    xs_f = _ln(h16).astype(bf16).astype(f32)
    xs = xs_f.astype(bf16)

    wg_copy.wait()
    wu_copy.wait()
    wd_copy.wait()
    g = jnp.dot(xs, wg_v[...], preferred_element_type=f32).astype(bf16).astype(f32)
    u = jnp.dot(xs, wu_v[...], preferred_element_type=f32).astype(bf16).astype(f32)
    a = ((g * jax.nn.sigmoid(g)).astype(bf16).astype(f32) * u).astype(bf16)
    y = jnp.dot(a, wd_v[...], preferred_element_type=f32).astype(bf16).astype(f32)
    r16 = lax.broadcasted_iota(jnp.int32, (16, 128), 0)
    gate = jax.nn.sigmoid(jnp.where(r16 == 0, rsel[0], rsel[1])).astype(bf16).astype(f32)
    y = (y * gate[:, 0:1]).astype(bf16).astype(f32)
    newrows = (h16 + (xs_f + y).astype(bf16).astype(f32)).astype(bf16).astype(f32)

    for i in range(NT):
        o_copy(i).wait()

    bases = []
    for c in range(2):
        base = pl.multiple_of((idx[c] // 16) * 16, 16)
        bases.append(base)
        blk = out_v[pl.ds(base, 16), :].astype(f32)
        nr = jnp.broadcast_to(newrows[c:c + 1, :], (16, D))
        out_v[pl.ds(base, 16), :] = jnp.where(row16 == idx[c] - base, nr, blk).astype(bf16)

    def fix_copy(c):
        rows = pl.ds(bases[c], 16)
        return pltpu.make_async_copy(out_v.at[rows], out_hbm.at[rows], sem_f.at[c])

    fix_copy(0).start()

    @pl.when(bases[0] != bases[1])
    def _():
        fix_copy(1).start()
        fix_copy(1).wait()

    fix_copy(0).wait()


@jax.jit
def pallas_sequential_preLN__linear_attn_block__moe_arch_mod__prompt_kernel(
    A_x: jax.Array,
    A_wqkv: jax.Array,
    A_wo: jax.Array,
    B_x: jax.Array,
    B_w_r: jax.Array,
    B_w_gate: jax.Array,
    B_w_up: jax.Array,
    B_w_down: jax.Array,
):
    any_spec = pl.BlockSpec(memory_space=pl.ANY)
    out = pl.pallas_call(
        _kernel,
        out_shape=jax.ShapeDtypeStruct((S, D), bf16),
        in_specs=[any_spec, any_spec, any_spec, pl.BlockSpec(memory_space=pltpu.VMEM),
                  any_spec, any_spec, any_spec],
        out_specs=any_spec,
        scratch_shapes=[
            pltpu.VMEM((S, D), bf16),
            pltpu.VMEM((D, 3 * D), bf16),
            pltpu.VMEM((D, D), bf16),
            pltpu.VMEM((D, F), bf16),
            pltpu.VMEM((D, F), bf16),
            pltpu.VMEM((F, D), bf16),
            pltpu.VMEM((S, D), bf16),
            pltpu.VMEM((D, D), bf16),
            pltpu.VMEM((NB, 128, 128), bf16),
            pltpu.VMEM((NB, 128, 128), f32),
            pltpu.VMEM((8, D), f32),
            pltpu.VMEM((S, D), f32),
            pltpu.VMEM((S, D), bf16),
            pltpu.VMEM((2 * NT, 128), f32),
            pltpu.VMEM((2 * NT, 128), jnp.int32),
            pltpu.SemaphoreType.DMA((NT,)),
            pltpu.SemaphoreType.DMA((7,)),
            pltpu.SemaphoreType.DMA((NT,)),
            pltpu.SemaphoreType.DMA((2,)),
        ],
        compiler_params=pltpu.CompilerParams(vmem_limit_bytes=100 * 1024 * 1024),
    )(A_x.reshape(S, D), A_wqkv, A_wo, B_w_r, B_w_gate, B_w_up, B_w_down)
    return out.reshape(1, S, D)
```

```python
import jax
import jax.numpy as jnp
from jax import lax
import jax.experimental.pallas as pl
import jax.experimental.pallas.tpu as pltpu

S, D, F, H = 2048, 1024, 3584, 32
TM = 512
NT = S // TM
NB = D // 128
KC = 256
NKC = D // KC
XC = 256
NXC = S // XC
SB = 32
FC = 512
NCH = 2
TILES = (512, 512, 512, 256, 256)
T2 = 512
NC2 = 256
NFC = F // FC
f32 = jnp.float32
bf16 = jnp.bfloat16


def _ln(x):
    m = jnp.mean(x, axis=-1, keepdims=True)
    xc = x - m
    v = jnp.mean(xc * xc, axis=-1, keepdims=True)
    return xc * lax.rsqrt(v + 1e-5)


class _Pace:
    def __init__(self, inf8):
        self.inf8 = inf8
        self.toks = []

    def ln(self, xb, paced=True):
        if paced and len(self.toks) >= NCH:
            g = jnp.where(self.toks[-NCH] > self.inf8, 1, 0).astype(jnp.uint32)
            g = jnp.tile(g, (xb.shape[0] // 16, xb.shape[1] // 128))
            xb = pltpu.bitcast(pltpu.bitcast(xb, jnp.uint32) | g, bf16)
        x = xb.astype(f32)
        m = jnp.mean(x, axis=-1, keepdims=True)
        xc = x - m
        v = jnp.mean(xc * xc, axis=-1, keepdims=True)
        rstd = lax.rsqrt(v + 1e-5)
        self.toks.append(jnp.broadcast_to(rstd[0:8], (8, 128)))
        return x, xc * rstd


def _phi(t):
    return jnp.where(t > 0, t + 1.0, jnp.exp(t)) + 1e-6


def _top2(r, iota, big):
    m1 = jnp.max(r, axis=0, keepdims=True)
    i1 = jnp.min(jnp.where(r == m1, iota, big), axis=0, keepdims=True)
    r2 = jnp.where(iota == i1, -jnp.inf, r)
    m2 = jnp.max(r2, axis=0, keepdims=True)
    i2 = jnp.min(jnp.where(r2 == m2, iota, big), axis=0, keepdims=True)
    return m1, i1, m2, i2


def _dot(a, b):
    return jnp.dot(a, b, preferred_element_type=f32)


def _kernel(x_hbm, wqkv_hbm, wo_hbm, wr_ref, wg_hbm, wu_hbm, wd_hbm, out_hbm,
            x_v, wqkv_v, wo_v, wg_v, wu_v, wd_v, ln1_v, pk_v, pqn_v, g_v, wp_v, zbd_v,
            h_v, out_v, r_v, sem_x, sem_k, sem_w, sem_o, sem_f):
    def x_copy(i):
        return pltpu.make_async_copy(x_hbm.at[pl.ds(i * XC, XC)], x_v.at[pl.ds(i * XC, XC)], sem_x.at[i])

    def k_copy(c):
        cs = pl.ds(D + c * KC, KC)
        return pltpu.make_async_copy(wqkv_hbm.at[:, cs], wqkv_v.at[:, cs], sem_k.at[c])

    def w_copy(j):
        return pltpu.make_async_copy(wqkv_hbm.at[:, pl.ds(j * D, D)], wqkv_v.at[:, pl.ds(j * D, D)], sem_w.at[j])

    wo_copy = pltpu.make_async_copy(wo_hbm, wo_v, sem_w.at[3])
    wg_copy = pltpu.make_async_copy(wg_hbm, wg_v, sem_w.at[4])
    wu_copy = pltpu.make_async_copy(wu_hbm, wu_v, sem_w.at[5])
    wd_copy = pltpu.make_async_copy(wd_hbm, wd_v, sem_w.at[6])

    def o_copy(i):
        rows = pl.ds(sum(TILES[:i]), TILES[i])
        return pltpu.make_async_copy(out_v.at[rows], out_hbm.at[rows], sem_o.at[i])

    rows = [slice(i * TM, (i + 1) * TM) for i in range(NT)]

    wr = wr_ref[...].astype(f32).reshape(1, D)
    pace = _Pace(jnp.broadcast_to(jnp.abs(wr[:, 0:128]) + jnp.inf, (8, 128)))

    def ln1(r0, n, paced=True):
        for s in range(r0, r0 + n, SB):
            ln1_v[s:s + SB, :] = pace.ln(x_v[s:s + SB, :], paced)[1].astype(bf16)

    zacc = [None] * NKC

    def kproj(r0, n, c):
        k = _dot(ln1_v[r0:r0 + n, :], wqkv_v[:, D + c * KC:D + (c + 1) * KC])
        pk = _phi(k).astype(bf16)
        pk_v[r0:r0 + n, c * KC:(c + 1) * KC] = pk
        zs = jnp.sum(pk.astype(f32).reshape(n // 8, 8, KC), axis=0)
        zacc[c] = zs if zacc[c] is None else zacc[c] + zs

    x_copy(0).start()
    k_copy(0).start()
    x_copy(0).wait()
    k_copy(1).start()
    ln1(0, XC, False)
    k_copy(0).wait()
    k_copy(2).start()
    kproj(0, XC, 0)
    k_copy(1).wait()
    k_copy(3).start()
    kproj(0, XC, 1)
    k_copy(2).wait()
    x_copy(1).start()
    kproj(0, XC, 2)
    k_copy(3).wait()
    x_copy(2).start()
    x_copy(3).start()
    kproj(0, XC, 3)
    x_copy(1).wait()
    ln1(XC, XC, False)
    for c in range(NKC):
        kproj(XC, XC, c)
        if c == 0:
            x_copy(2).wait()
            x_copy(4).start()
            x_copy(5).start()
        if c == 2:
            x_copy(3).wait()
        if c < 2:
            ln1(2 * XC + c * 128, 128)
        else:
            ln1(3 * XC + (c - 2) * 128, 128)
    for i in range(1, NT):
        for c in range(NKC):
            kproj(i * TM, TM, c)
            if i == 1 and c == 0:
                x_copy(6).start()
                x_copy(7).start()
                w_copy(2).start()
                w_copy(0).start()
                wo_copy.start()
            if i == 2 and c == 0:
                wg_copy.start()
                wu_copy.start()
                wd_copy.start()
            if i + 1 < NT:
                if c == 0:
                    x_copy(2 * i + 2).wait()
                if c == 2:
                    x_copy(2 * i + 3).wait()
                ln1((i + 1) * TM + c * 128, 128)
    zrow = jnp.sum(jnp.concatenate(zacc, axis=1), axis=0, keepdims=True)

    for j in range(NB):
        cs = slice(j * 128, (j + 1) * 128)
        g_v[cs, :] = lax.dot_general(pk_v[:, cs], ln1_v[...], (((0,), (0,)), ((), ())),
                                     preferred_element_type=f32).astype(bf16)

    w_copy(2).wait()
    w_copy(0).wait()
    wo_copy.wait()
    ri = lax.broadcasted_iota(jnp.int32, (128, 128), 0) // 32
    ci = lax.broadcasted_iota(jnp.int32, (128, 128), 1) // 32
    mask = ri == ci
    for j in range(NB):
        cs = slice(j * 128, (j + 1) * 128)
        kv = _dot(g_v[cs, :], wqkv_v[:, 2 * D + j * 128:2 * D + (j + 1) * 128])
        kvb = jnp.where(mask, kv, 0.0).astype(bf16)
        wp_v[cs, :] = _dot(kvb, wo_v[cs, :]).astype(bf16)
        zcol = jnp.transpose(jnp.broadcast_to(zrow[:, cs], (128, 128)))
        zbd_v[j] = jnp.where(mask, zcol, 0.0).astype(bf16)

    def stage_a(r0, nr, c0, nc):
        rs = slice(r0, r0 + nr)
        a = ln1_v[rs, :]
        q = _dot(a, wqkv_v[:, c0:c0 + nc])
        pq = _phi(q).astype(bf16)
        for jj in range(nc // 128):
            j = c0 // 128 + jj
            pqj = pq[:, jj * 128:(jj + 1) * 128]
            den = _dot(pqj, zbd_v[j]) + 1e-6
            pqn_v[rs, j * 128:(j + 1) * 128] = (pqj.astype(f32) * pl.reciprocal(den, approx=True)).astype(bf16)

    def stage_b(r0, nr, c0, nc):
        rs = slice(r0, r0 + nr)
        cs = slice(c0, c0 + nc)
        attn = _dot(pqn_v[rs, :], wp_v[:, cs])
        h_v[rs, cs] = (x_v[rs, cs].astype(f32) + attn).astype(bf16)

    def stage_c(r0, n, paced):
        for s in range(r0, r0 + n, SB):
            h, ln2 = pace.ln(h_v[s:s + SB, :], paced)
            out_v[s:s + SB, :] = (h + ln2).astype(bf16)
            r = jnp.sum(ln2 * wr, axis=-1, keepdims=True).astype(bf16).astype(f32)
            r_v[s:s + SB, :] = jnp.broadcast_to(r, (SB, 128))

    N2 = len(TILES)
    st = [sum(TILES[:i]) for i in range(N2)]
    for c in range(0, D, NC2):
        stage_a(0, TILES[0], c, NC2)
    for i in range(N2):
        if i + 1 < N2:
            for c in range(0, D, NC2):
                stage_a(st[i + 1], TILES[i + 1], c, NC2)
        for c in range(0, D, NC2):
            stage_b(st[i], TILES[i], c, NC2)
        stage_c(st[i], TILES[i], i + 1 < N2)
        o_copy(i).start()

    iota = lax.broadcasted_iota(jnp.int32, (S, 128), 0)
    m1, i1, m2, i2 = _top2(r_v[...], iota, 1 << 30)
    idx = [jnp.clip(i1[0, 0], 0, S - 1), jnp.clip(i2[0, 0], 0, S - 1)]
    rsel = [m1, m2]

    row16 = lax.broadcasted_iota(jnp.int32, (16, D), 0)
    bases = [pl.multiple_of((idx[c] // 16) * 16, 16) for c in range(2)]
    hh = [jnp.sum(jnp.where(row16 == idx[c] - bases[c], h_v[pl.ds(bases[c], 16), :].astype(f32), 0.0),
                  axis=0, keepdims=True) for c in range(2)]
    h16 = jnp.where(row16 == 0, hh[0], jnp.where(row16 == 1, hh[1], 0.0))
    xs_f = _ln(h16).astype(bf16).astype(f32)
    xs = xs_f.astype(bf16)

    wg_copy.wait()
    wu_copy.wait()
    wd_copy.wait()
    y = None
    for c in range(NFC):
        cs = slice(c * FC, (c + 1) * FC)
        g = _dot(xs, wg_v[:, cs]).astype(bf16).astype(f32)
        u = _dot(xs, wu_v[:, cs]).astype(bf16).astype(f32)
        a = ((g * jax.nn.sigmoid(g)).astype(bf16).astype(f32) * u).astype(bf16)
        yc = _dot(a, wd_v[cs, :])
        y = yc if y is None else y + yc
    y = y.astype(bf16).astype(f32)
    r16 = lax.broadcasted_iota(jnp.int32, (16, 128), 0)
    gate = jax.nn.sigmoid(jnp.where(r16 == 0, rsel[0], rsel[1])).astype(bf16).astype(f32)
    y = (y * gate[:, 0:1]).astype(bf16).astype(f32)
    newrows = (h16 + (xs_f + y).astype(bf16).astype(f32)).astype(bf16).astype(f32)

    for i in range(N2):
        o_copy(i).wait()

    for c in range(2):
        base = bases[c]
        blk = out_v[pl.ds(base, 16), :].astype(f32)
        nr = jnp.broadcast_to(newrows[c:c + 1, :], (16, D))
        out_v[pl.ds(base, 16), :] = jnp.where(row16 == idx[c] - base, nr, blk).astype(bf16)

    def fix_copy(c):
        rows_ = pl.ds(bases[c], 16)
        return pltpu.make_async_copy(out_v.at[rows_], out_hbm.at[rows_], sem_f.at[c])

    fix_copy(0).start()

    @pl.when(bases[0] != bases[1])
    def _():
        fix_copy(1).start()
        fix_copy(1).wait()

    fix_copy(0).wait()


@jax.jit
def pallas_sequential_preLN__linear_attn_block__moe_arch_mod__prompt_kernel(
    A_x: jax.Array,
    A_wqkv: jax.Array,
    A_wo: jax.Array,
    B_x: jax.Array,
    B_w_r: jax.Array,
    B_w_gate: jax.Array,
    B_w_up: jax.Array,
    B_w_down: jax.Array,
):
    any_spec = pl.BlockSpec(memory_space=pl.ANY)
    out = pl.pallas_call(
        _kernel,
        out_shape=jax.ShapeDtypeStruct((S, D), bf16),
        in_specs=[any_spec, any_spec, any_spec, pl.BlockSpec(memory_space=pltpu.VMEM),
                  any_spec, any_spec, any_spec],
        out_specs=any_spec,
        scratch_shapes=[
            pltpu.VMEM((S, D), bf16),
            pltpu.VMEM((D, 3 * D), bf16),
            pltpu.VMEM((D, D), bf16),
            pltpu.VMEM((D, F), bf16),
            pltpu.VMEM((D, F), bf16),
            pltpu.VMEM((F, D), bf16),
            pltpu.VMEM((S, D), bf16),
            pltpu.VMEM((S, D), bf16),
            pltpu.VMEM((S, D), bf16),
            pltpu.VMEM((D, D), bf16),
            pltpu.VMEM((D, D), bf16),
            pltpu.VMEM((NB, 128, 128), bf16),
            pltpu.VMEM((S, D), bf16),
            pltpu.VMEM((S, D), bf16),
            pltpu.VMEM((S, 128), f32),
            pltpu.SemaphoreType.DMA((NXC,)),
            pltpu.SemaphoreType.DMA((NKC,)),
            pltpu.SemaphoreType.DMA((7,)),
            pltpu.SemaphoreType.DMA((len(TILES),)),
            pltpu.SemaphoreType.DMA((2,)),
        ],
        compiler_params=pltpu.CompilerParams(vmem_limit_bytes=100 * 1024 * 1024),
    )(A_x.reshape(S, D), A_wqkv, A_wo, B_w_r, B_w_gate, B_w_up, B_w_down)
    return out.reshape(1, S, D)
```

```python
import jax
import jax.numpy as jnp
from jax import lax
import jax.experimental.pallas as pl
import jax.experimental.pallas.tpu as pltpu

S, D, F, H = 2048, 1024, 3584, 32
TM = 512
NT = S // TM
NB = D // 128
KC = 256
NKC = D // KC
XC = 256
NXC = S // XC
SB = 32
FC = 512
NCH = 2
TILES = (512, 512, 512, 256, 256)
T2 = 512
NC2 = 256
NFC = F // FC
f32 = jnp.float32
bf16 = jnp.bfloat16


def _ln(x):
    m = jnp.mean(x, axis=-1, keepdims=True)
    xc = x - m
    v = jnp.mean(xc * xc, axis=-1, keepdims=True)
    return xc * lax.rsqrt(v + 1e-5)


class _Pace:
    def __init__(self, inf8):
        self.inf8 = inf8
        self.toks = []

    def ln(self, xb, paced=True):
        if paced and len(self.toks) >= NCH:
            g = jnp.where(self.toks[-NCH] > self.inf8, 1, 0).astype(jnp.uint32)
            g = jnp.tile(g, (xb.shape[0] // 16, xb.shape[1] // 128))
            xb = pltpu.bitcast(pltpu.bitcast(xb, jnp.uint32) | g, bf16)
        x = xb.astype(f32)
        m = jnp.mean(x, axis=-1, keepdims=True)
        xc = x - m
        v = jnp.mean(xc * xc, axis=-1, keepdims=True)
        rstd = lax.rsqrt(v + 1e-5)
        self.toks.append(jnp.broadcast_to(rstd[0:8], (8, 128)))
        return x, xc * rstd


def _phi(t):
    return jnp.where(t > 0, t + 1.0, jnp.exp(t)) + 1e-6


def _top2(r, iota, big):
    m1 = jnp.max(r, axis=0, keepdims=True)
    i1 = jnp.min(jnp.where(r == m1, iota, big), axis=0, keepdims=True)
    r2 = jnp.where(iota == i1, -jnp.inf, r)
    m2 = jnp.max(r2, axis=0, keepdims=True)
    i2 = jnp.min(jnp.where(r2 == m2, iota, big), axis=0, keepdims=True)
    return m1, i1, m2, i2


u32 = jnp.uint32


def _ld(ref, r0, nr, cs=slice(None)):
    return pltpu.bitcast(ref[r0 // 2:(r0 + nr) // 2, cs], bf16)


def _st(ref, r0, cs, val):
    ref[r0 // 2:(r0 + val.shape[0]) // 2, cs] = pltpu.bitcast(val.astype(bf16), u32)


def _dot(a, b):
    return jnp.dot(a, b, preferred_element_type=f32)


def _kernel(x_hbm, wqkv_hbm, wo_hbm, wr_ref, wg_hbm, wu_hbm, wd_hbm, out_hbm,
            x_v, wqkv_v, wo_v, wg_v, wu_v, wd_v, ln1_v, pk_v, pqn_v, g_v, wp_v, zbd_v,
            h_v, out_v, sem_x, sem_k, sem_w, sem_o, sem_f):
    def x_copy(i):
        return pltpu.make_async_copy(x_hbm.at[pl.ds(i * XC, XC)], x_v.at[pl.ds(i * XC, XC)], sem_x.at[i])

    def k_copy(c):
        cs = pl.ds(D + c * KC, KC)
        return pltpu.make_async_copy(wqkv_hbm.at[:, cs], wqkv_v.at[:, cs], sem_k.at[c])

    def w_copy(j):
        return pltpu.make_async_copy(wqkv_hbm.at[:, pl.ds(j * D, D)], wqkv_v.at[:, pl.ds(j * D, D)], sem_w.at[j])

    wo_copy = pltpu.make_async_copy(wo_hbm, wo_v, sem_w.at[3])
    wg_copy = pltpu.make_async_copy(wg_hbm.bitcast(u32), wg_v, sem_w.at[4])
    wu_copy = pltpu.make_async_copy(wu_hbm.bitcast(u32), wu_v, sem_w.at[5])
    wd_copy = pltpu.make_async_copy(wd_hbm.bitcast(u32), wd_v, sem_w.at[6])

    def o_copy(i):
        rows = pl.ds(sum(TILES[:i]), TILES[i])
        return pltpu.make_async_copy(out_v.at[rows], out_hbm.at[rows], sem_o.at[i])

    rows = [slice(i * TM, (i + 1) * TM) for i in range(NT)]

    wr = wr_ref[...].astype(f32).reshape(1, D)
    pace = _Pace(jnp.broadcast_to(jnp.abs(wr[:, 0:128]) + jnp.inf, (8, 128)))

    def ln1(r0, n, paced=True):
        for s in range(r0, r0 + n, SB):
            _st(ln1_v, s, slice(None), pace.ln(x_v[s:s + SB, :], paced)[1])

    zacc = [None] * NKC

    def kproj(r0, n, c):
        k = _dot(_ld(ln1_v, r0, n), wqkv_v[:, D + c * KC:D + (c + 1) * KC])
        pk = _phi(k).astype(bf16)
        _st(pk_v, r0, slice(c * KC, (c + 1) * KC), pk)
        zs = jnp.sum(pk.astype(f32).reshape(n // 8, 8, KC), axis=0)
        zacc[c] = zs if zacc[c] is None else zacc[c] + zs

    x_copy(0).start()
    k_copy(0).start()
    x_copy(0).wait()
    k_copy(1).start()
    ln1(0, XC, False)
    k_copy(0).wait()
    k_copy(2).start()
    kproj(0, XC, 0)
    k_copy(1).wait()
    k_copy(3).start()
    kproj(0, XC, 1)
    k_copy(2).wait()
    x_copy(1).start()
    kproj(0, XC, 2)
    k_copy(3).wait()
    x_copy(2).start()
    x_copy(3).start()
    kproj(0, XC, 3)
    x_copy(1).wait()
    ln1(XC, XC, False)
    for c in range(NKC):
        kproj(XC, XC, c)
        if c == 0:
            x_copy(2).wait()
            x_copy(4).start()
            x_copy(5).start()
        if c == 2:
            x_copy(3).wait()
        if c < 2:
            ln1(2 * XC + c * 128, 128)
        else:
            ln1(3 * XC + (c - 2) * 128, 128)
    for i in range(1, NT):
        for c in range(NKC):
            kproj(i * TM, TM, c)
            if i == 1 and c == 0:
                x_copy(6).start()
                x_copy(7).start()
                w_copy(2).start()
                w_copy(0).start()
                wo_copy.start()
            if i == 2 and c == 0:
                wg_copy.start()
                wu_copy.start()
                wd_copy.start()
            if i + 1 < NT:
                if c == 0:
                    x_copy(2 * i + 2).wait()
                if c == 2:
                    x_copy(2 * i + 3).wait()
                ln1((i + 1) * TM + c * 128, 128)
    zrow = jnp.sum(jnp.concatenate(zacc, axis=1), axis=0, keepdims=True)

    GW = 512
    for j in range(D // GW):
        cs = slice(j * GW, (j + 1) * GW)
        _st(g_v, j * GW, slice(None), lax.dot_general(
            _ld(pk_v, 0, S, cs), _ld(ln1_v, 0, S), (((0,), (0,)), ((), ())), preferred_element_type=f32))

    w_copy(2).wait()
    w_copy(0).wait()
    wo_copy.wait()
    ri = lax.broadcasted_iota(jnp.int32, (128, 128), 0) // 32
    ci = lax.broadcasted_iota(jnp.int32, (128, 128), 1) // 32
    mask = ri == ci
    for j in range(NB):
        cs = slice(j * 128, (j + 1) * 128)
        kv = _dot(_ld(g_v, j * 128, 128), wqkv_v[:, 2 * D + j * 128:2 * D + (j + 1) * 128])
        kvb = jnp.where(mask, kv, 0.0).astype(bf16)
        _st(wp_v, j * 128, slice(None), _dot(kvb, wo_v[cs, :]))
        zcol = jnp.transpose(jnp.broadcast_to(zrow[:, cs], (128, 128)))
        zbd_v[j] = jnp.where(mask, zcol, 0.0).astype(bf16)

    def stage_a(r0, nr, c0, nc):
        rs = slice(r0, r0 + nr)
        a = _ld(ln1_v, r0, nr)
        q = _dot(a, wqkv_v[:, c0:c0 + nc])
        pq = _phi(q).astype(bf16)
        for jj in range(nc // 128):
            j = c0 // 128 + jj
            pqj = pq[:, jj * 128:(jj + 1) * 128]
            den = _dot(pqj, zbd_v[j]) + 1e-6
            _st(pqn_v, r0, slice(j * 128, (j + 1) * 128), pqj.astype(f32) * pl.reciprocal(den, approx=True))

    def stage_b(r0, nr, c0, nc):
        rs = slice(r0, r0 + nr)
        cs = slice(c0, c0 + nc)
        attn = _dot(_ld(pqn_v, r0, nr), _ld(wp_v, 0, D, cs))
        h_v[rs, cs] = (x_v[rs, cs].astype(f32) + attn).astype(bf16)

    sub8 = lax.broadcasted_iota(jnp.int32, (8, 128), 0)
    ninf = jnp.full((8, 128), -jnp.inf, f32)
    best = [ninf, sub8, ninf, sub8 + 8]

    def stage_c(r0, n, paced):
        for s in range(r0, r0 + n, SB):
            h, ln2 = pace.ln(h_v[s:s + SB, :], paced)
            out_v[s:s + SB, :] = (h + ln2).astype(bf16)
            r = jnp.sum(ln2 * wr, axis=-1, keepdims=True).astype(bf16).astype(f32)
            rb = jnp.broadcast_to(r, (SB, 128))
            for t in range(0, SB, 8):
                v, ix = rb[t:t + 8], sub8 + (s + t)
                b1, j1, b2, j2 = best
                w1, w2 = v > b1, v > b2
                best[:] = (jnp.where(w1, v, b1), jnp.where(w1, ix, j1),
                           jnp.where(w1, b1, jnp.where(w2, v, b2)), jnp.where(w1, j1, jnp.where(w2, ix, j2)))

    N2 = len(TILES)
    st = [sum(TILES[:i]) for i in range(N2)]
    for c in range(0, D, NC2):
        stage_a(0, TILES[0], c, NC2)
    for i in range(N2):
        if i + 1 < N2:
            for c in range(0, D, NC2):
                stage_a(st[i + 1], TILES[i + 1], c, NC2)
        for c in range(0, D, NC2):
            stage_b(st[i], TILES[i], c, NC2)
        stage_c(st[i], TILES[i], i + 1 < N2)
        o_copy(i).start()

    m1, i1, m2, i2 = _top2(jnp.concatenate([best[0], best[2]], axis=0),
                           jnp.concatenate([best[1], best[3]], axis=0), 1 << 30)
    idx = [jnp.clip(i1[0, 0], 0, S - 1), jnp.clip(i2[0, 0], 0, S - 1)]
    rsel = [m1, m2]

    row16 = lax.broadcasted_iota(jnp.int32, (16, D), 0)
    bases = [pl.multiple_of((idx[c] // 16) * 16, 16) for c in range(2)]
    hh = [jnp.sum(jnp.where(row16 == idx[c] - bases[c], h_v[pl.ds(bases[c], 16), :].astype(f32), 0.0),
                  axis=0, keepdims=True) for c in range(2)]
    h16 = jnp.where(row16 == 0, hh[0], jnp.where(row16 == 1, hh[1], 0.0))
    xs_f = _ln(h16).astype(bf16).astype(f32)
    xs = xs_f.astype(bf16)

    wg_copy.wait()
    wu_copy.wait()
    wd_copy.wait()
    y = None
    for c in range(NFC):
        cs = slice(c * FC, (c + 1) * FC)
        g = _dot(xs, _ld(wg_v, 0, D, cs)).astype(bf16).astype(f32)
        u = _dot(xs, _ld(wu_v, 0, D, cs)).astype(bf16).astype(f32)
        a = ((g * jax.nn.sigmoid(g)).astype(bf16).astype(f32) * u).astype(bf16)
        yc = _dot(a, _ld(wd_v, c * FC, FC))
        y = yc if y is None else y + yc
    y = y.astype(bf16).astype(f32)
    r16 = lax.broadcasted_iota(jnp.int32, (16, 128), 0)
    gate = jax.nn.sigmoid(jnp.where(r16 == 0, rsel[0], rsel[1])).astype(bf16).astype(f32)
    y = (y * gate[:, 0:1]).astype(bf16).astype(f32)
    newrows = (h16 + (xs_f + y).astype(bf16).astype(f32)).astype(bf16).astype(f32)

    for i in range(N2):
        o_copy(i).wait()

    for c in range(2):
        base = bases[c]
        blk = out_v[pl.ds(base, 16), :].astype(f32)
        nr = jnp.broadcast_to(newrows[c:c + 1, :], (16, D))
        out_v[pl.ds(base, 16), :] = jnp.where(row16 == idx[c] - base, nr, blk).astype(bf16)

    def fix_copy(c):
        rows_ = pl.ds(bases[c], 16)
        return pltpu.make_async_copy(out_v.at[rows_], out_hbm.at[rows_], sem_f.at[c])

    fix_copy(0).start()

    @pl.when(bases[0] != bases[1])
    def _():
        fix_copy(1).start()
        fix_copy(1).wait()

    fix_copy(0).wait()


@jax.jit
def pallas_sequential_preLN__linear_attn_block__moe_arch_mod__prompt_kernel(
    A_x: jax.Array,
    A_wqkv: jax.Array,
    A_wo: jax.Array,
    B_x: jax.Array,
    B_w_r: jax.Array,
    B_w_gate: jax.Array,
    B_w_up: jax.Array,
    B_w_down: jax.Array,
):
    any_spec = pl.BlockSpec(memory_space=pl.ANY)
    out = pl.pallas_call(
        _kernel,
        out_shape=jax.ShapeDtypeStruct((S, D), bf16),
        in_specs=[any_spec, any_spec, any_spec, pl.BlockSpec(memory_space=pltpu.VMEM),
                  any_spec, any_spec, any_spec],
        out_specs=any_spec,
        scratch_shapes=[
            pltpu.VMEM((S, D), bf16),
            pltpu.VMEM((D, 3 * D), bf16),
            pltpu.VMEM((D, D), bf16),
            pltpu.VMEM((D // 2, F), u32),
            pltpu.VMEM((D // 2, F), u32),
            pltpu.VMEM((F // 2, D), u32),
            pltpu.VMEM((S // 2, D), u32),
            pltpu.VMEM((S // 2, D), u32),
            pltpu.VMEM((S // 2, D), u32),
            pltpu.VMEM((D // 2, D), u32),
            pltpu.VMEM((D // 2, D), u32),
            pltpu.VMEM((NB, 128, 128), bf16),
            pltpu.VMEM((S, D), bf16),
            pltpu.VMEM((S, D), bf16),
            pltpu.SemaphoreType.DMA((NXC,)),
            pltpu.SemaphoreType.DMA((NKC,)),
            pltpu.SemaphoreType.DMA((7,)),
            pltpu.SemaphoreType.DMA((len(TILES),)),
            pltpu.SemaphoreType.DMA((2,)),
        ],
        compiler_params=pltpu.CompilerParams(vmem_limit_bytes=100 * 1024 * 1024),
    )(A_x.reshape(S, D), A_wqkv, A_wo, B_w_r, B_w_gate, B_w_up, B_w_down)
    return out.reshape(1, S, D)
```
